```python
import jax
import jax.numpy as jnp

def _softmax(x, axis=-1):
    return jax.nn.softmax(x, axis=axis)
def _gelu(x):
    return jax.nn.gelu(x, approximate=True)
def _silu(x):
    return jax.nn.silu(x)
def _sigmoid(x):
    return jax.nn.sigmoid(x)
def _layernorm(x, axis=-1, eps=1e-5):
    m = jnp.mean(x, axis=axis, keepdims=True)
    v = jnp.var(x, axis=axis, keepdims=True)
    return (x - m) / jnp.sqrt(v + eps)
def _scatter_add(tgt, idx, src, axis=0):
    return tgt.at[idx].add(src)
def _segment_sum(src, seg, n):
    return jax.ops.segment_sum(src, seg, n)
class _Rng:
    def __init__(self, key):
        self._k = key
    def _next(self):
        self._k, sub = jax.random.split(self._k)
        return sub
    def normal(self, shape):
        return jax.random.normal(self._next(), shape, dtype=jnp.bfloat16)
    def randint(self, lo, hi, shape):
        return jax.random.randint(self._next(), shape, lo, hi, dtype=jnp.int32)
    def uniform(self, shape, lo=0.0, hi=1.0):
        return jax.random.uniform(self._next(), shape, jnp.bfloat16, lo, hi)
    def permutation(self, n):
        return jax.random.permutation(self._next(), n)


kernel_name = 'standalone__winograd__vision'

def setup_inputs():
    _rng = _Rng(jax.random.key(int.from_bytes(__import__("os").urandom(4), "little")))
    _w = (lambda a: (lambda t: t.astype(jnp.bfloat16) if jnp.issubdtype(t.dtype, jnp.floating) else t)(jnp.asarray(a)))
    H = W = 512 // 2 * 2
    C = 192
    return {
        "x": _w((lambda *s: _rng.normal(s) * 0.05)(1, H, W, C)),
        "w": _w((lambda *s: _rng.normal(s) * 0.05)(3, 3, C, C)),
    }

def reference(x, w):
    N, H, W, C = x.shape
    K = w.shape[-1]
    G  = jnp.array([[1.0,0.0,0.0],[0.5,0.5,0.5],[0.5,-0.5,0.5],[0.0,0.0,1.0]], dtype=x.dtype)
    Bt = jnp.array([[1.0,0.0,-1.0,0.0],[0.0,1.0,1.0,0.0],[0.0,-1.0,1.0,0.0],[0.0,1.0,0.0,-1.0]], dtype=x.dtype)
    At = jnp.array([[1.0,1.0,1.0,0.0],[0.0,1.0,-1.0,-1.0]], dtype=x.dtype)
    U = jnp.einsum("ar,rsck,bs->abck", G, w, G)
    xp = jnp.pad(x, ((0,0),(1,1),(1,1),(0,0)))
    nH, nW = H // 2, W // 2
    patches = []
    for i in range(4):
        for j in range(4):
            patches.append(xp[:, i:i + 2 * nH:2, j:j + 2 * nW:2, :])
    d = jnp.stack(patches).reshape(4, 4, N * nH * nW, C)
    V = jnp.einsum("ai,ijpc,bj->abpc", Bt, d, Bt)
    M = jnp.einsum("abck,abpc->abpk", U, V)
    Y = jnp.einsum("ma,abpk,nb->pmnk", At, M, At)
    Y = Y.reshape(N, nH, nW, 2, 2, K)
    Y = (lambda x, *d: x.transpose(*d))(Y, 0, 1, 3, 2, 4, 5).reshape(N, H, W, K)
    return Y
```

```python
import jax
import jax.numpy as jnp
from jax import lax
import jax.experimental.pallas as pl
import jax.experimental.pallas.tpu as pltpu

R = 16
CC = 16

_G = (
    (1 / 4, 0.0, 0.0),
    (-1 / 6, -1 / 6, -1 / 6),
    (-1 / 6, 1 / 6, -1 / 6),
    (1 / 24, 1 / 12, 1 / 6),
    (1 / 24, -1 / 12, 1 / 6),
    (0.0, 0.0, 1.0),
)


def _kernel(x_ref, top_ref, bot_ref, w_ref, o_ref, ut_ref, v_ref, m_ref):
    i = pl.program_id(0)
    n = pl.num_programs(0)
    C = x_ref.shape[1]
    W = x_ref.shape[2]
    f32 = jnp.float32
    bf16 = jnp.bfloat16

    @pl.when(i == 0)
    def _():
        for a in range(6):
            for s in range(3):
                u = sum(_G[a][r] * w_ref[r, s].astype(f32) for r in range(3) if _G[a][r] != 0.0)
                ut_ref[a, :, s * C:(s + 1) * C] = u.T.astype(bf16)

    lane = lax.broadcasted_iota(jnp.int32, (CC, W), 1)
    top_scale = jnp.where(i > 0, 1.0, 0.0).astype(f32)
    bot_scale = jnp.where(i < n - 1, 1.0, 0.0).astype(f32)

    for g in range(R // 4):
        def row(j, c0):
            r = 4 * g + j - 1
            if r < 0:
                return top_ref[0, pl.ds(c0, CC), :].astype(f32) * top_scale
            if r >= R:
                return bot_ref[0, pl.ds(c0, CC), :].astype(f32) * bot_scale
            return x_ref[r, pl.ds(c0, CC), :].astype(f32)

        def in_body(cb, carry):
            c0 = pl.multiple_of(cb * CC, CC)
            d0, d1, d2, d3, d4, d5 = (row(j, c0) for j in range(6))
            t1 = d4 - 4.0 * d2
            t2 = d3 - 4.0 * d1
            t3 = d4 - d2
            t4 = d3 - d1
            t42 = t4 + t4
            vs = (
                4.0 * (d0 - d2) + t3,
                t1 + t2,
                t1 - t2,
                t3 + t42,
                t3 - t42,
                (d5 - d3) - 4.0 * t4,
            )
            for a, v in enumerate(vs):
                vl = jnp.where(lane == 0, 0.0, pltpu.roll(v, 1, 1))
                vr = jnp.where(lane == W - 1, 0.0, pltpu.roll(v, W - 1, 1))
                v_ref[a, pl.ds(c0, CC), :] = vl.astype(bf16)
                v_ref[a, pl.ds(C + c0, CC), :] = v.astype(bf16)
                v_ref[a, pl.ds(2 * C + c0, CC), :] = vr.astype(bf16)
            return carry

        lax.fori_loop(0, C // CC, in_body, 0)

        for a in range(6):
            m_ref[a] = jnp.dot(ut_ref[a], v_ref[a], preferred_element_type=f32)

        def out_body(cb, carry):
            c0 = pl.multiple_of(cb * CC, CC)
            m0, m1, m2, m3, m4, m5 = (m_ref[a, pl.ds(c0, CC), :] for a in range(6))
            s12 = m1 + m2
            d12 = m1 - m2
            s34 = m3 + m4
            d34 = m3 - m4
            o_ref[4 * g + 0, pl.ds(c0, CC), :] = (m0 + s12 + s34).astype(bf16)
            o_ref[4 * g + 1, pl.ds(c0, CC), :] = (d12 + 2.0 * d34).astype(bf16)
            o_ref[4 * g + 2, pl.ds(c0, CC), :] = (s12 + 4.0 * s34).astype(bf16)
            o_ref[4 * g + 3, pl.ds(c0, CC), :] = (d12 + 8.0 * d34 + m5).astype(bf16)
            return carry

        lax.fori_loop(0, C // CC, out_body, 0)


@jax.jit
def pallas_standalone__winograd__vision_kernel(x: jax.Array, w: jax.Array):
    N, H, W, C = x.shape
    K = w.shape[-1]
    xt = jnp.transpose(x, (0, 1, 3, 2)).reshape(H, C, W)
    nb = H // R
    out = pl.pallas_call(
        _kernel,
        grid=(nb,),
        in_specs=[
            pl.BlockSpec((R, C, W), lambda i: (i, 0, 0)),
            pl.BlockSpec((1, C, W), lambda i: (jnp.maximum(i * R - 1, 0), 0, 0)),
            pl.BlockSpec((1, C, W), lambda i: (jnp.minimum(i * R + R, H - 1), 0, 0)),
            pl.BlockSpec((3, 3, C, K), lambda i: (0, 0, 0, 0)),
        ],
        out_specs=pl.BlockSpec((R, K, W), lambda i: (i, 0, 0)),
        out_shape=jax.ShapeDtypeStruct((H, K, W), x.dtype),
        scratch_shapes=[
            pltpu.VMEM((6, K, 3 * C), jnp.bfloat16),
            pltpu.VMEM((6, 3 * C, W), jnp.bfloat16),
            pltpu.VMEM((6, K, W), jnp.float32),
        ],
        compiler_params=pltpu.CompilerParams(
            dimension_semantics=("arbitrary",),
            vmem_limit_bytes=100 * 1024 * 1024,
        ),
    )(xt, xt, xt, w)
    return jnp.transpose(out.reshape(N, H, K, W), (0, 1, 3, 2))
```

```python
import jax
import jax.numpy as jnp
from jax import lax
import jax.experimental.pallas as pl
import jax.experimental.pallas.tpu as pltpu

R = 16
CC = 16

_G = (
    (1 / 4, 0.0, 0.0),
    (-1 / 6, -1 / 6, -1 / 6),
    (-1 / 6, 1 / 6, -1 / 6),
    (1 / 24, 1 / 12, 1 / 6),
    (1 / 24, -1 / 12, 1 / 6),
    (0.0, 0.0, 1.0),
)


def _kernel(x_ref, nxt_ref, w_ref, o_ref, ut_ref, v0_ref, v1_ref, m0_ref, m1_ref):
    i = pl.program_id(0)
    n = pl.num_programs(0)
    C = x_ref.shape[1]
    W = x_ref.shape[2]
    f32 = jnp.float32
    bf16 = jnp.bfloat16
    G = R // 4
    NCH = C // CC
    v_refs = (v0_ref, v1_ref)
    m_refs = (m0_ref, m1_ref)
    lane = lax.broadcasted_iota(jnp.int32, (CC, W), 1)
    last = i == n - 1

    def in_chunk(g, cb):
        c0 = cb * CC
        v_ref = v_refs[g % 2]

        def row(j):
            r = 4 * g + j - 1
            if r < 0:
                return jnp.zeros((CC, W), f32)
            if r >= R:
                d = nxt_ref[r - R, c0:c0 + CC, :].astype(f32)
                return jnp.where(last, 0.0, d) if r == R and g < G else d
            return x_ref[r, c0:c0 + CC, :].astype(f32)

        d0, d1, d2, d3, d4, d5 = (row(j) for j in range(6))
        t1 = d4 - 4.0 * d2
        t2 = d3 - 4.0 * d1
        t3 = d4 - d2
        t4 = d3 - d1
        t42 = t4 + t4
        vs = (
            4.0 * (d0 - d2) + t3,
            t1 + t2,
            t1 - t2,
            t3 + t42,
            t3 - t42,
            (d5 - d3) - 4.0 * t4,
        )
        for a, v in enumerate(vs):
            vb = v.astype(bf16)
            p = pltpu.bitcast(vb, jnp.uint32)
            ln = lane[:CC // 2]
            pl_ = jnp.where(ln == 0, jnp.uint32(0), pltpu.roll(p, 1, 1))
            pr_ = jnp.where(ln == W - 1, jnp.uint32(0), pltpu.roll(p, W - 1, 1))
            h = CC // 2
            v_ref[a, c0 // 2:c0 // 2 + h, :] = pl_
            v_ref[a, (C + c0) // 2:(C + c0) // 2 + h, :] = p
            v_ref[a, (2 * C + c0) // 2:(2 * C + c0) // 2 + h, :] = pr_

    def mm(g, a):
        v = pltpu.bitcast(v_refs[g % 2][a], bf16)
        m_refs[g % 2][a] = jnp.dot(ut_ref[a], v, preferred_element_type=f32)

    def out_chunk(g, cb):
        c0 = cb * CC
        m_ref = m_refs[g % 2]
        m0, m1, m2, m3, m4, m5 = (m_ref[a, c0:c0 + CC, :] for a in range(6))
        s12 = m1 + m2
        d12 = m1 - m2
        s34 = m3 + m4
        d34 = m3 - m4
        o_ref[4 * g + 0, c0:c0 + CC, :] = (m0 + s12 + s34).astype(bf16)
        o_ref[4 * g + 1, c0:c0 + CC, :] = (d12 + 2.0 * d34).astype(bf16)
        o_ref[4 * g + 2, c0:c0 + CC, :] = (s12 + 4.0 * s34).astype(bf16)
        o_ref[4 * g + 3, c0:c0 + CC, :] = (d12 + 8.0 * d34 + m5).astype(bf16)

    @pl.when(i == 0)
    def _():
        for a in range(6):
            for s in range(3):
                u = sum(_G[a][r] * w_ref[r, s].astype(f32) for r in range(3) if _G[a][r] != 0.0)
                ut_ref[a, :, s * C:(s + 1) * C] = u.T.astype(bf16)
        for cb in range(NCH):
            in_chunk(0, cb)

    for g in range(G):
        for a in range(6):
            mm(g, a)
            for cb in range(a * NCH // 6, (a + 1) * NCH // 6):
                in_chunk(g + 1, cb)
                if g > 0:
                    out_chunk(g - 1, cb)
    for cb in range(NCH):
        out_chunk(G - 1, cb)


@jax.jit
def pallas_standalone__winograd__vision_kernel(x: jax.Array, w: jax.Array):
    N, H, W, C = x.shape
    K = w.shape[-1]
    xt = jnp.transpose(x, (0, 1, 3, 2)).reshape(H, C, W)
    nb = H // R
    out = pl.pallas_call(
        _kernel,
        grid=(nb,),
        in_specs=[
            pl.BlockSpec((R, C, W), lambda i: (i, 0, 0)),
            pl.BlockSpec((8, C, W), lambda i: (jnp.minimum((i + 1) * (R // 8), H // 8 - 1), 0, 0)),
            pl.BlockSpec((3, 3, C, K), lambda i: (0, 0, 0, 0)),
        ],
        out_specs=pl.BlockSpec((R, K, W), lambda i: (i, 0, 0)),
        out_shape=jax.ShapeDtypeStruct((H, K, W), x.dtype),
        scratch_shapes=[
            pltpu.VMEM((6, K, 3 * C), jnp.bfloat16),
            pltpu.VMEM((6, 3 * C // 2, W), jnp.uint32),
            pltpu.VMEM((6, 3 * C // 2, W), jnp.uint32),
            pltpu.VMEM((6, K, W), jnp.float32),
            pltpu.VMEM((6, K, W), jnp.float32),
        ],
        compiler_params=pltpu.CompilerParams(
            dimension_semantics=("arbitrary",),
            vmem_limit_bytes=100 * 1024 * 1024,
        ),
    )(xt, xt, w)
    return jnp.transpose(out.reshape(N, H, K, W), (0, 1, 3, 2))
```

```python
import jax
import jax.numpy as jnp
from jax import lax
import jax.experimental.pallas as pl
import jax.experimental.pallas.tpu as pltpu

R = 12
CC = 16

_PTS = (0.0, 1.0, -1.0, 2.0, -2.0, 0.5, -0.5)


def _g_row(p):
    f = 1.0
    for q in _PTS:
        if q != p:
            f *= p - q
    return (1.0 / f, p / f, p * p / f)


_G = ((1.0, 0.0, 0.0),) + tuple(_g_row(p) for p in _PTS[1:]) + ((0.0, 0.0, 1.0),)


def _kernel(rem, x_ref, nxt_ref, nx2_ref, w_ref, o_ref, ut_ref, v0_ref, v1_ref, m0_ref, m1_ref):
    i = pl.program_id(0)
    n = pl.num_programs(0)
    C = x_ref.shape[1]
    W = x_ref.shape[2]
    f32 = jnp.float32
    bf16 = jnp.bfloat16
    G = R // 6
    NCH = C // CC
    v_refs = (v0_ref, v1_ref)
    m_refs = (m0_ref, m1_ref)
    lane = lax.broadcasted_iota(jnp.int32, (CC, W), 1)
    last = i == n - 1

    def in_chunk(g, cb):
        c0 = cb * CC
        v_ref = v_refs[g % 2]

        def row(j):
            r = 6 * g + j - 1
            if r < 0:
                return jnp.zeros((CC, W), f32)
            if r >= R:
                d = (nxt_ref if r < R + 4 else nx2_ref)[(r - R) % 4, c0:c0 + CC, :].astype(f32)
                return jnp.where(last, 0.0, d) if r == R and g < G else d
            d = x_ref[r, c0:c0 + CC, :].astype(f32)
            return jnp.where(last, 0.0, d) if r >= rem else d

        d0, d1, d2, d3, d4, d5, d6, d7 = (row(j) for j in range(8))
        e1 = d2 + d6 - 4.25 * d4
        o1 = d1 + d5 - 4.25 * d3
        q4 = 1.25 * d4
        q3 = 2.5 * d3
        e2 = d6 + 0.25 * d2 - q4
        o2 = 0.5 * d1 - q3 + (d5 + d5)
        e3 = d6 + 4.0 * (d2 - q4)
        o3 = (d1 + d1) - q3 + 0.5 * d5
        vs = (
            d0 - d6 + 5.25 * (d4 - d2),
            e1 + o1, e1 - o1, e2 + o2, e2 - o2, e3 + o3, e3 - o3,
            d7 - d1 + 5.25 * (d3 - d5),
        )
        for a, v in enumerate(vs):
            vb = v.astype(bf16)
            p = pltpu.bitcast(vb, jnp.uint32)
            ln = lane[:CC // 2]
            pl_ = jnp.where(ln == 0, jnp.uint32(0), pltpu.roll(p, 1, 1))
            pr_ = jnp.where(ln == W - 1, jnp.uint32(0), pltpu.roll(p, W - 1, 1))
            h = CC // 2
            v_ref[a, c0 // 2:c0 // 2 + h, :] = pl_
            v_ref[a, (C + c0) // 2:(C + c0) // 2 + h, :] = p
            v_ref[a, (2 * C + c0) // 2:(2 * C + c0) // 2 + h, :] = pr_

    def mm(g, a):
        v = pltpu.bitcast(v_refs[g % 2][a], bf16)
        m_refs[g % 2][a] = jnp.dot(ut_ref[a], v, preferred_element_type=f32)

    def out_chunk(g, cb):
        c0 = cb * CC
        m_ref = m_refs[g % 2]
        m0, m1, m2, m3, m4, m5, m6, m7 = (m_ref[a, c0:c0 + CC, :] for a in range(8))
        s1, t1 = m1 + m2, m1 - m2
        s2, t2 = m3 + m4, m3 - m4
        s3, t3 = m5 + m6, m5 - m6
        ys = (
            m0 + s1 + s2 + s3,
            t1 + 2.0 * t2 + 0.5 * t3,
            s1 + 4.0 * s2 + 0.25 * s3,
            t1 + 8.0 * t2 + 0.125 * t3,
            s1 + 16.0 * s2 + 0.0625 * s3,
            t1 + 32.0 * t2 + 0.03125 * t3 + m7,
        )
        for j, y in enumerate(ys):
            o_ref[6 * g + j, c0:c0 + CC, :] = y.astype(bf16)

    @pl.when(i == 0)
    def _():
        for a in range(8):
            for s in range(3):
                u = sum(_G[a][r] * w_ref[r, s].astype(f32) for r in range(3) if _G[a][r] != 0.0)
                ut_ref[a, :, s * C:(s + 1) * C] = u.T.astype(bf16)
        for cb in range(NCH):
            in_chunk(0, cb)

    for g in range(G):
        for a in range(8):
            mm(g, a)
            for cb in range(a * NCH // 8, (a + 1) * NCH // 8):
                in_chunk(g + 1, cb)
                if g > 0:
                    out_chunk(g - 1, cb)
    for cb in range(NCH):
        out_chunk(G - 1, cb)


@jax.jit
def pallas_standalone__winograd__vision_kernel(x: jax.Array, w: jax.Array):
    N, H, W, C = x.shape
    K = w.shape[-1]
    xt = jnp.transpose(x, (0, 1, 3, 2)).reshape(H, C, W)
    nb = pl.cdiv(H, R)
    out = pl.pallas_call(
        lambda *a: _kernel(H - (nb - 1) * R, *a),
        grid=(nb,),
        in_specs=[
            pl.BlockSpec((R, C, W), lambda i: (i, 0, 0)),
            pl.BlockSpec((4, C, W), lambda i: (jnp.minimum((i + 1) * (R // 4), H // 4 - 1), 0, 0)),
            pl.BlockSpec((4, C, W), lambda i: (jnp.minimum((i + 1) * (R // 4) + 1, H // 4 - 1), 0, 0)),
            pl.BlockSpec((3, 3, C, K), lambda i: (0, 0, 0, 0)),
        ],
        out_specs=pl.BlockSpec((R, K, W), lambda i: (i, 0, 0)),
        out_shape=jax.ShapeDtypeStruct((H, K, W), x.dtype),
        scratch_shapes=[
            pltpu.VMEM((8, K, 3 * C), jnp.bfloat16),
            pltpu.VMEM((8, 3 * C // 2, W), jnp.uint32),
            pltpu.VMEM((8, 3 * C // 2, W), jnp.uint32),
            pltpu.VMEM((8, K, W), jnp.float32),
            pltpu.VMEM((8, K, W), jnp.float32),
        ],
        compiler_params=pltpu.CompilerParams(
            dimension_semantics=("arbitrary",),
            vmem_limit_bytes=100 * 1024 * 1024,
        ),
    )(xt, xt, xt, w)
    return jnp.transpose(out.reshape(N, H, K, W), (0, 1, 3, 2))
```
